```python
import os as _os
_os.environ.setdefault("JAX_PLATFORMS", "cpu")
import jax
import jax.numpy as jnp

def _softmax(x, axis=-1):
    return jax.nn.softmax(x, axis=axis)
def _gelu(x):
    return jax.nn.gelu(x, approximate=True)
def _silu(x):
    return jax.nn.silu(x)
def _sigmoid(x):
    return jax.nn.sigmoid(x)
def _layernorm(x, axis=-1, eps=1e-5):
    m = jnp.mean(x, axis=axis, keepdims=True)
    v = jnp.var(x, axis=axis, keepdims=True)
    return (x - m) / jnp.sqrt(v + eps)
def _scatter_add(tgt, idx, src, axis=0):
    return tgt.at[idx].add(src)
def _segment_sum(src, seg, n):
    return jax.ops.segment_sum(src, seg, n)
class _Rng:
    def __init__(self, key):
        self._k = key
    def _next(self):
        self._k, sub = jax.random.split(self._k)
        return sub
    def normal(self, shape):
        return jax.random.normal(self._next(), shape, dtype=jnp.bfloat16)
    def randint(self, lo, hi, shape):
        return jax.random.randint(self._next(), shape, lo, hi, dtype=jnp.int32)
    def uniform(self, shape, lo=0.0, hi=1.0):
        return jax.random.uniform(self._next(), shape, jnp.bfloat16, lo, hi)
    def permutation(self, n):
        return jax.random.permutation(self._next(), n)


kernel_name = 'concat_heads__mha_block_cached__mha_block_cached__near_ridge'

def setup_inputs():
    _rng = _Rng(jax.random.key(int.from_bytes(__import__("os").urandom(4), "little")))
    _w = (lambda a: (lambda t: t.astype(jnp.bfloat16) if jnp.issubdtype(t.dtype, jnp.floating) else t)(jnp.asarray(a)))
    def _A_setup():
        B, Sq, D = 16, 80, 512
        H, Sk, Dh = 32, 80, 128
        return {
            "x": _w((lambda *s: _rng.normal(s) * 0.8)(B, Sq, D)),
            "k_cache": _w((lambda *s: _rng.normal(s) * 0.8)(B, H, Sk, Dh)),
            "v_cache": _w((lambda *s: _rng.normal(s) * 0.05)(B, H, Sk, Dh)),
            "wq": _w((lambda *s: _rng.normal(s) * 0.8)(D, H * Dh) * (D ** -0.5)),
            "wo": _w((lambda *s: _rng.normal(s) * 0.05)(H * Dh, D) * ((H * Dh) ** -0.5)),
        }
    _A_in = _A_setup()

    def _B_setup():
        B, Sq, D = 16, 80, 512
        H, Sk, Dh = 32, 80, 128
        return {
            "x": _w((lambda *s: _rng.normal(s) * 0.8)(B, Sq, D)),
            "k_cache": _w((lambda *s: _rng.normal(s) * 0.8)(B, H, Sk, Dh)),
            "v_cache": _w((lambda *s: _rng.normal(s) * 0.05)(B, H, Sk, Dh)),
            "wq": _w((lambda *s: _rng.normal(s) * 0.8)(D, H * Dh) * (D ** -0.5)),
            "wo": _w((lambda *s: _rng.normal(s) * 0.05)(H * Dh, D) * ((H * Dh) ** -0.5)),
        }
    _B_in = _B_setup()

    return {
        "A_x": _A_in["x"],
        "A_k_cache": _A_in["k_cache"],
        "A_v_cache": _A_in["v_cache"],
        "A_wq": _A_in["wq"],
        "A_wo": _A_in["wo"],
        "B_x": _B_in["x"],
        "B_k_cache": _B_in["k_cache"],
        "B_v_cache": _B_in["v_cache"],
        "B_wq": _B_in["wq"],
        "B_wo": _B_in["wo"],
    }

def reference(A_x, A_k_cache, A_v_cache, A_wq, A_wo, B_x, B_k_cache, B_v_cache, B_wq, B_wo):
    def _A_ref(x, k_cache, v_cache, wq, wo):
        B, Sq, D = x.shape
        H, Dh = 32, 128
        q = (lambda x, *d: x.transpose(*d))((x @ wq).reshape(B, Sq, H, Dh), 0, 2, 1, 3)
        scores = jnp.einsum("bhqd,bhkd->bhqk", q, k_cache) * (Dh ** -0.5)
        p = _softmax(scores, axis=-1)
        o = jnp.einsum("bhqk,bhkd->bhqd", p, v_cache)
        return (lambda x, *d: x.transpose(*d))(o, 0, 2, 1, 3).reshape(B, Sq, H * Dh) @ wo

    def _B_ref(x, k_cache, v_cache, wq, wo):
        B, Sq, D = x.shape
        H, Dh = 32, 128
        q = (lambda x, *d: x.transpose(*d))((x @ wq).reshape(B, Sq, H, Dh), 0, 2, 1, 3)
        scores = jnp.einsum("bhqd,bhkd->bhqk", q, k_cache) * (Dh ** -0.5)
        p = _softmax(scores, axis=-1)
        o = jnp.einsum("bhqk,bhkd->bhqd", p, v_cache)
        return (lambda x, *d: x.transpose(*d))(o, 0, 2, 1, 3).reshape(B, Sq, H * Dh) @ wo

    a = _A_ref(A_x, A_k_cache, A_v_cache, A_wq, A_wo)
    b = _B_ref(B_x, B_k_cache, B_v_cache, B_wq, B_wo)
    return jnp.concatenate([a, b], axis=-1)
```

```python
import contextlib

import jax
import jax.numpy as jnp
import jax.experimental.pallas as pl
import jax.experimental.pallas.tpu as pltpu

B, S, D, H, SK, DH = 16, 80, 512, 32, 80, 128
M = B * S
T = 128
NB = 4
NC = B // NB
R = NB * S
NQUAD = H // NB
NSTEP = NQUAD // 2
NP = 49
LOG2E = 1.4426950408889634
f32, bf16, u32 = jnp.float32, jnp.bfloat16, jnp.uint32


def _quad(m):
    n = len(m) // 2
    return ([r[:n] for r in m[:n]], [r[n:] for r in m[:n]], [r[:n] for r in m[n:]], [r[n:] for r in m[n:]])


def _add(a, b):
    return [[x + y for x, y in zip(r, s)] for r, s in zip(a, b)]


def _sub(a, b):
    return [[x - y for x, y in zip(r, s)] for r, s in zip(a, b)]


def left_operands(m):
    if len(m) == 1:
        return [m[0][0]]
    a11, a12, a21, a22 = _quad(m)
    parts = (_add(a11, a22), _add(a21, a22), a11, a22, _add(a11, a12), _sub(a21, a11), _sub(a12, a22))
    return [x for t in parts for x in left_operands(t)]


def right_operands(m):
    if len(m) == 1:
        return [m[0][0]]
    b11, b12, b21, b22 = _quad(m)
    parts = (_add(b11, b22), b11, _sub(b12, b22), _sub(b21, b11), b22, _add(b11, b12), _add(b21, b22))
    return [x for t in parts for x in right_operands(t)]


def combine(ps):
    if len(ps) == 1:
        return [[ps[0]]]
    n = len(ps) // 7
    m1, m2, m3, m4, m5, m6, m7 = [combine(ps[i * n:(i + 1) * n]) for i in range(7)]
    c11 = _add(_sub(_add(m1, m4), m5), m7)
    c12 = _add(m3, m5)
    c21 = _add(m2, m4)
    c22 = _add(_add(_sub(m1, m2), m3), m6)
    return [r + s for r, s in zip(c11, c12)] + [r + s for r, s in zip(c21, c22)]


class _Terms:
    def __init__(self, t):
        self.t = t

    def __add__(self, o):
        return _Terms({**self.t, **o.t})

    def __sub__(self, o):
        return _Terms({**self.t, **{k: -v for k, v in o.t.items()}})


W_TERMS = [sorted(x.t.items()) for x in right_operands([[_Terms({(i, j): 1}) for j in range(NB)] for i in range(NB)])]


def product_order(spec):
    d = [int(ch) - 1 for ch in str(spec)[1:]]
    return [7 * a + b for a in d for b in d] if str(spec)[0] == "8" else [7 * a + b for b in d for a in d]


def issue_order(q_groups, attend, lagp, lago, tail, gq, go, qfirst, ag, pq, po, qmode, skew):
    qs = [("Q", c, u, p) for u in q_groups for c in range(NC) for p in product_order(pq)]
    if qmode:
        qs = [("Q", c, u, p) for c in range(NC) for u in q_groups for p in product_order(pq)]
    ev = []
    if attend:
        total = 20 * (len(qs) + 2 * NC * NP + 4 * B * NB)
        t0 = 20 * NC * NP if qfirst else skew
        period = (total - t0 - 40 * NP - tail) / NC
        n = 2 * NB * NB // ag
        for c in range(NC):
            for j in range(n):
                at = t0 + (c + j / n) * period
                ev.append((at, 20 * ag, ("K", c, j * ag)))
                ev.append((at + lagp, 20 * ag, ("P", c, j * ag)))
            done = t0 + (c + 1 - 1 / n) * period + lagp
            ev.append((done + 1, 0, ("o", c)))
            span = period if c < NC - 1 else 40 * NP
            for rank, p in enumerate(product_order(po)):
                ev.append((done + lago + (rank + 0.5) / NP * span, 40, ("O", c, p)))
            ev.append((done + lago + span, 0, ("F", c)))
    ev.sort(key=lambda e: e[0])
    out, held, cum = [], [], 0

    def emit_q():
        t = qs.pop(0)
        out.append(t)
        if not qs or qs[0][1:3] != t[1:3]:
            out.append(("q",) + t[1:3])

    for at, cost, t in ev:
        while len(qs) >= gq and cum + 10 * gq <= at:
            for _ in range(gq):
                emit_q()
            cum += 20 * gq
        if t[0] == "K" and t[2] >= NB * NB:
            while ("q", t[1], 1) not in out:
                emit_q()
                cum += 20
        if t[0] == "O" or (held and t[0] == "F"):
            held.append(t)
            if sum(h[0] == "O" for h in held) == go:
                out += held
                held = []
                cum += 40 * go
        else:
            out.append(t)
            cum += cost
    while qs:
        emit_q()
    return out + held


def build(lagp=600, lago=400, tail=3000, pq=82413567, po=82534671, qmode=0, skew=0, nx0=2, LA=dict(lago=200, tail=2000, gq=1), FB={}, L=dict(lago=200, tail=500, gq=1), F=dict(lago=500, tail=1500, gq=1), gq=2, go=1, ag=4, lp=0, pkx=0, pkq=1, scopes=False, only=0):
    def order(q_groups, attend, qfirst=False, **kw):
        a = dict(lagp=lagp, lago=lago, tail=tail, gq=gq, go=go, ag=ag, pq=pq, po=po, qmode=qmode, skew=skew)
        a.update(kw)
        return issue_order(q_groups, attend, qfirst=qfirst, **a)
    sc = (lambda n: jax.named_scope(n)) if scopes else (lambda n: contextlib.nullcontext())

    def kernel(ax, ak, av, awq, awo, bx, bk, bv, bwq, bwo, out,
               xb, kb, vb, wqb, wob, xc, qb, acc, ob, xsem, kvsem, wsem, osem):
        srcs = ((ax, ak, av, awq, awo), (bx, bk, bv, bwq, bwo))

        def heads(g, n):
            return pl.ds(g * n if isinstance(g, int) else pl.multiple_of(g * n, n), n)

        def copy(kind, br, i, half=0):
            x, k, v, wq, wo = srcs[br]
            if kind == "x":
                return pltpu.make_async_copy(x.at[pl.ds(i * R, R)], xb.at[br, pl.ds(i * R, R)], xsem.at[br, i])
            if kind in "kv":
                src, dst = (k, kb) if kind == "k" else (v, vb)
                rows = pl.ds(half * (B // 2), B // 2)
                return pltpu.make_async_copy(src.at[rows, heads(i, 2 * NB)], dst.at[br * NSTEP + i, rows],
                                             kvsem.at[br * NSTEP + i, 2 * "kv".index(kind) + half])
            if kind == "q":
                return pltpu.make_async_copy(wq.at[:, heads(i, D)], wqb.at[br * NQUAD + i], wsem.at[br, i])
            return pltpu.make_async_copy(wo.at[heads(i, 2 * D)], wob.at[br * NSTEP + i], wsem.at[br, NQUAD + i])

        def step_copies(br, t):
            return ([copy("q", br, 2 * t + 1)] + [copy(kind, br, t, 0) for kind in "kv"]
                    + [copy("o", br, t)] + [copy(kind, br, t, 1) for kind in "kv"])

        def out_copy(br, c):
            return pltpu.make_async_copy(ob.at[br, pl.ds(c * R, R)], out.at[pl.ds(c * R, R), heads(br, D)], osem.at[br, c])

        def rows16(ref, idx):
            return pltpu.bitcast(ref.bitcast(u32)[idx], bf16)

        def put(ref, idx, v, as_words):
            ref[idx] = pltpu.bitcast(v.astype(bf16), u32) if as_words else v.astype(bf16)

        def get(ref, idx, as_words):
            return pltpu.bitcast(ref[idx], bf16) if as_words else rows16(ref, idx)

        def weight_operand(ref, slot, row0, p):
            def block(ij):
                return ref[slot, row0 + ij[0] * T:row0 + (ij[0] + 1) * T, ij[1] * T:(ij[1] + 1) * T]

            def signed_sum(terms):
                if len(terms) == 1:
                    return block(terms[0][0]).astype(f32), terms[0][1]
                (u, su), (v, sv) = signed_sum(terms[:len(terms) // 2]), signed_sum(terms[len(terms) // 2:])
                return (u + v, su) if su == sv else ((u - v, 1) if su > 0 else (v - u, 1))

            if len(W_TERMS[p]) == 1:
                return block(W_TERMS[p][0][0])
            total, sign = signed_sum(W_TERMS[p])
            assert sign > 0
            return total

        def run(tasks, br, t, fresh=False, last=False, new_x=None, hooks=()):
            hooks, x_done = dict(hooks), set()
            wq_ops, wo_ops, q_prod, q_val, probs, heads_out, o_ops, o_prod = {}, {}, {}, {}, {}, {}, {}, {}
            for task in tasks:
                if task in hooks:
                    hooks[task]()
                kind, c = task[:2]
                if kind == "Q":
                    u, p = task[2:]
                    xbr = br if new_x is None or u == 1 else new_x
                    if new_x is not None and u == 2 and c not in x_done:
                        x_done.add(c)
                        x = [[xb[new_x, c * R + i * S:c * R + (i + 1) * S, j * T:(j + 1) * T].astype(f32)
                              for j in range(NB)] for i in range(NB)]
                        for p2, v in enumerate(left_operands(x)):
                            put(xc, (new_x, c, p2), v, pkx == 0)
                    if (u, p) not in wq_ops:
                        wq_ops[u, p] = weight_operand(wqb, br * NQUAD + 2 * t + u, 0, p).astype(bf16)
                    q_prod[c, u, p] = jnp.dot(get(xc, (xbr, c, p), pkx == 0), wq_ops[u, p], preferred_element_type=f32)
                elif kind == "q":
                    u = task[2]
                    q = combine([q_prod[c, u, p] for p in range(NP)])
                    for i in range(NB):
                        for h in range(NB):
                            if u == 1:
                                q_val[c, i, h] = q[i][h].astype(bf16)
                            else:
                                put(qb, ((t + 1) % 2, c * NB + i, h), q[i][h], pkq == 0)
                elif kind == "K":
                    for j in range(task[2], task[2] + ag):
                        u, i, h = j // (NB * NB), j // NB % NB, j % NB
                        q = q_val[c, i, h] if u else get(qb, (t % 2, c * NB + i, h), pkq == 0)
                        k = rows16(kb, (br * NSTEP + t, c * NB + i, u * NB + h))
                        s = jax.lax.dot_general(q, k, (((1,), (1,)), ((), ())), preferred_element_type=f32)
                        e = jnp.exp2((s - jnp.max(s, axis=-1, keepdims=True)) * (DH ** -0.5 * LOG2E))
                        probs[c, j] = (e * pl.reciprocal(jnp.sum(e, axis=-1, keepdims=True), approx=True)).astype(bf16)
                elif kind == "P":
                    for j in range(task[2], task[2] + ag):
                        u, i, h = j // (NB * NB), j // NB % NB, j % NB
                        v = rows16(vb, (br * NSTEP + t, c * NB + i, u * NB + h))
                        heads_out[c, u, i, h] = jnp.dot(probs[c, j], v, preferred_element_type=f32)
                elif kind == "o":
                    ops = [left_operands([[heads_out[c, u, i, h] for h in range(NB)] for i in range(NB)]) for u in range(2)]
                    o_ops[c] = [jnp.concatenate(pair, axis=1).astype(bf16) for pair in zip(*ops)]
                elif kind == "O":
                    p = task[2]
                    if p not in wo_ops:
                        wo_ops[p] = jnp.concatenate([weight_operand(wob, br * NSTEP + t, u * D, p) for u in range(2)], axis=0).astype(bf16)
                    r = jnp.dot(o_ops[c][p], wo_ops[p], preferred_element_type=f32)
                    if not fresh:
                        r = r + acc[c, p]
                    if last:
                        o_prod[c, p] = r
                    else:
                        acc[c, p] = r
                elif last:
                    res = combine([o_prod[c, p] for p in range(NP)])
                    for i in range(NB):
                        for j in range(NB):
                            ob[br, c * R + i * S:c * R + (i + 1) * S, j * T:(j + 1) * T] = res[i][j].astype(bf16)
                    out_copy(br, c).start()

        def wait(name, cps, then=()):
            def hook():
                with sc(name):
                    for cp in cps:
                        cp.wait()
                for cp in then:
                    cp.start()
            return hook

        def middle(br):
            def body(t, carry):
                with sc("mid"):
                    for cp in step_copies(br, t) + [copy("q", br, 2 * t + 2)]:
                        cp.wait()
                    for cp in step_copies(br, t + 1):
                        cp.start()

                    @pl.when(t + 1 < NSTEP - 1)
                    def _():
                        copy("q", br, 2 * t + 4).start()

                    if br == 0:
                        @pl.when(t + 1 == NSTEP - 1)
                        def _():
                            for cp in [copy("q", 1, 0)] + [copy("x", 1, c) for c in range(NC)]:
                                cp.start()
                    run(order((1, 2), True), br, t)
                return carry
            jax.lax.fori_loop(1, NSTEP - 1, body, 0)

        if only:
            def one(t, _):
                if only == 2: run(order((1,), True, **L), t, NSTEP - 1, last=True)
                if only == 3: run(order((2,), False), t, -1, new_x=0)
                if only == 5: run(order((1, 2), True, **LA), 0, t, last=True, new_x=1)
                if only == 6: run(order((1, 2), True, **FB), 0, t, fresh=True)
                if only == 4: run(order((1, 2), True, qfirst=True, **F), t, 0, fresh=True)
                return 0
            if only == 1: middle(0)
            else: jax.lax.fori_loop(0, 2, one, 0)
            out_copy(0, 0).start(); out_copy(0, 0).wait()
            return
        x = [[copy("x", br, c) for c in range(NC)] for br in range(2)]
        wq0 = [copy("q", br, 0) for br in range(2)]
        first, second = step_copies(0, 0), step_copies(0, 1)
        p0 = product_order(pq)[0]
        for cp in [wq0[0]] + x[0][:nx0]:
            cp.start()
        with sc("pro"):
            run(order((2,), False), 0, -1, new_x=0, hooks={
                ("Q", 0, 2, p0): wait("s_h0", [wq0[0], x[0][0]], x[0][nx0:] + first[:1] + [copy("q", 0, 2)]),
                ("Q", 1, 2, p0): wait("s_h1", x[0][1:2], first[1:4]),
                ("Q", 2, 2, p0): wait("s_h2", x[0][2:], first[4:])})
        with sc("first"):
            wait("s_h3", [first[0], copy("q", 0, 2)], second[:4] + [copy("q", 0, 4)])()
            run(order((1, 2), True, qfirst=True, **F), 0, 0, fresh=True, hooks={
                ("K", 0, 0): wait("s_h4", first[1:4], second[4:]),
                ("K", NC // 2, 0): wait("s_h5", first[4:])})
        middle(0)
        with sc("last"):
            wait("s_l", step_copies(0, NSTEP - 1) + [wq0[1]] + x[1], step_copies(1, 0) + [copy("q", 1, 2)])()
            run(order((1, 2), True, **LA), 0, NSTEP - 1, last=True, new_x=1)
        with sc("first"):
            wait("s_l", step_copies(1, 0) + [copy("q", 1, 2)], step_copies(1, 1) + [copy("q", 1, 4)])()
            run(order((1, 2), True, **FB), 1, 0, fresh=True)
        middle(1)
        with sc("last"):
            wait("s_l", step_copies(1, NSTEP - 1))()
            run(order((1,), True, **L), 1, NSTEP - 1, last=True)
        with sc("epi"):
            for br in range(2):
                for c in range(NC):
                    out_copy(br, c).wait()

    def fn(ax, ak, av, awq, awo, bx, bk, bv, bwq, bwo):
        words = lambda shape, w: pltpu.VMEM(shape[:-2] + (shape[-2] // 2, shape[-1]), u32) if w else pltpu.VMEM(shape, bf16)
        out = pl.pallas_call(
            kernel,
            out_shape=jax.ShapeDtypeStruct((M, 2 * D), bf16),
            in_specs=[pl.BlockSpec(memory_space=pl.ANY)] * 10,
            out_specs=pl.BlockSpec(memory_space=pl.ANY),
            scratch_shapes=[
                pltpu.VMEM((2, M, D), bf16),
                pltpu.VMEM((2 * NSTEP, B, 2 * NB, SK, DH), bf16), pltpu.VMEM((2 * NSTEP, B, 2 * NB, SK, DH), bf16),
                pltpu.VMEM((2 * NQUAD, D, NB * DH), bf16), pltpu.VMEM((2 * NSTEP, 2 * NB * DH, D), bf16),
                words((2, NC, NP, S, T), pkx == 0), words((2, B, NB, S, DH), pkq == 0),
                pltpu.VMEM((NC, NP, S, T), f32),
                pltpu.VMEM((2, M, D), bf16),
                pltpu.SemaphoreType.DMA((2, NC)), pltpu.SemaphoreType.DMA((2 * NSTEP, 4)),
                pltpu.SemaphoreType.DMA((2, NQUAD + NSTEP)), pltpu.SemaphoreType.DMA((2, NC)),
            ],
            compiler_params=pltpu.CompilerParams(
                vmem_limit_bytes=110 * 1024 * 1024, disable_bounds_checks=True,
                flags={"XLA_TPU_MAX_INSTS_TO_PREDICATE": lp} if lp else None),
        )(ax.reshape(M, D), ak, av, awq, awo, bx.reshape(M, D), bk, bv, bwq, bwo)
        return out.reshape(B, S, 2 * D)
    return fn


@jax.jit
def pallas_concat_heads__mha_block_cached__mha_block_cached__near_ridge_kernel(
    A_x, A_k_cache, A_v_cache, A_wq, A_wo, B_x, B_k_cache, B_v_cache, B_wq, B_wo,
):
    return build()(A_x, A_k_cache, A_v_cache, A_wq, A_wo, B_x, B_k_cache, B_v_cache, B_wq, B_wo)
```

```python
import jax
import jax.numpy as jnp
import jax.experimental.pallas as pl
import jax.experimental.pallas.tpu as pltpu

B, S, D, H, SK, DH = 16, 80, 512, 32, 80, 128
M = B * S
T = 128
NB = 4
NC = B // NB
R = NB * S
NQUAD = H // NB
NSTEP = NQUAD // 2
NP = 49
LOG2E = 1.4426950408889634
f32, bf16, u32 = jnp.float32, jnp.bfloat16, jnp.uint32


def _quad(m):
    n = len(m) // 2
    return ([r[:n] for r in m[:n]], [r[n:] for r in m[:n]], [r[:n] for r in m[n:]], [r[n:] for r in m[n:]])


def _add(a, b):
    return [[x + y for x, y in zip(r, s)] for r, s in zip(a, b)]


def _sub(a, b):
    return [[x - y for x, y in zip(r, s)] for r, s in zip(a, b)]


def left_operands(m):
    if len(m) == 1:
        return [m[0][0]]
    a11, a12, a21, a22 = _quad(m)
    parts = (_add(a11, a22), _add(a21, a22), a11, a22, _add(a11, a12), _sub(a21, a11), _sub(a12, a22))
    return [x for t in parts for x in left_operands(t)]


def right_operands(m):
    if len(m) == 1:
        return [m[0][0]]
    b11, b12, b21, b22 = _quad(m)
    parts = (_add(b11, b22), b11, _sub(b12, b22), _sub(b21, b11), b22, _add(b11, b12), _add(b21, b22))
    return [x for t in parts for x in right_operands(t)]


def combine(ps):
    if len(ps) == 1:
        return [[ps[0]]]
    n = len(ps) // 7
    m1, m2, m3, m4, m5, m6, m7 = [combine(ps[i * n:(i + 1) * n]) for i in range(7)]
    c11 = _add(_sub(_add(m1, m4), m5), m7)
    c12 = _add(m3, m5)
    c21 = _add(m2, m4)
    c22 = _add(_add(_sub(m1, m2), m3), m6)
    return [r + s for r, s in zip(c11, c12)] + [r + s for r, s in zip(c21, c22)]


class _Terms:
    def __init__(self, t):
        self.t = t

    def __add__(self, o):
        return _Terms({**self.t, **o.t})

    def __sub__(self, o):
        return _Terms({**self.t, **{k: -v for k, v in o.t.items()}})


W_TERMS = [sorted(x.t.items()) for x in right_operands([[_Terms({(i, j): 1}) for j in range(NB)] for i in range(NB)])]


def product_order(spec):
    d = [int(ch) - 1 for ch in str(spec)]
    return [7 * a + b for a in d for b in d]


def issue_order(q_groups, attend, lagp, lago, tail, gq, go, pq, po, skew, spanf):
    qs = [("Q", c, u, p) for u in q_groups for c in range(NC) for p in product_order(pq)]
    ev = []
    if attend:
        total = 20 * (len(qs) + 2 * NC * NP + 4 * B * NB)
        t0 = skew
        period = (total - t0 - 40 * NP - tail) / NC
        n = 2 * NB * NB // NB
        for c in range(NC):
            for j in range(n):
                at = t0 + (c + j / n) * period
                ev.append((at, 20 * NB, ("K", c, j * NB)))
                ev.append((at + lagp, 20 * NB, ("P", c, j * NB)))
            done = t0 + (c + 1 - 1 / n) * period + lagp
            ev.append((done + 1, 0, ("o", c)))
            span = spanf * period if c < NC - 1 else 40 * NP
            for rank, p in enumerate(product_order(po)):
                ev.append((done + lago + (rank + 0.5) / NP * span, 40, ("O", c, p)))
            ev.append((done + lago + span, 0, ("F", c)))
    ev.sort(key=lambda e: e[0])
    out, held, cum = [], [], 0

    def emit_q():
        t = qs.pop(0)
        out.append(t)
        if not qs or qs[0][1:3] != t[1:3]:
            out.append(("q",) + t[1:3])

    for at, cost, t in ev:
        while len(qs) >= gq and cum + 10 * gq <= at:
            for _ in range(gq):
                emit_q()
            cum += 20 * gq
        if t[0] == "K" and t[2] >= NB * NB:
            while 1 in q_groups and ("q", t[1], 1) not in out:
                emit_q()
                cum += 20
        if t[0] == "O" or (held and t[0] == "F"):
            held.append(t)
            if sum(h[0] == "O" for h in held) == go:
                out += held
                held = []
                cum += 40 * go
        else:
            out.append(t)
            cum += cost
    while qs:
        emit_q()
    return out + held


PLAIN = dict(lagp=600, lago=650, tail=3300, gq=1, go=1, pq=3524167, po=3425671, skew=0, spanf=1.1)
F = dict(lagp=600, lago=200, tail=1200, spanf=1.2)
M1 = dict(lagp=600, lago=500, tail=3800, go=2, spanf=1.0)
FB = dict(lagp=600, lago=500, tail=3800, go=2, pq=2413567, spanf=1.2)
LA = dict(lagp=600, lago=300, tail=2200, gq=2, go=2, pq=2413567, spanf=1.0, skew=200)
L = dict(lagp=550, lago=300, tail=-600, gq=2, go=2, pq=2413567, spanf=1.0)


def order(q_groups, attend, **kw):
    return issue_order(q_groups, attend, **{**PLAIN, **kw})


def build():
    def kernel(ax, ak, av, awq, awo, bx, bk, bv, bwq, bwo, out,
               xb, kb, vb, wqb, wob, xc, qb, acc, ob, xsem, kvsem, wsem, osem):
        srcs = ((ax, ak, av, awq, awo), (bx, bk, bv, bwq, bwo))

        def heads(g, n):
            return pl.ds(g * n if isinstance(g, int) else pl.multiple_of(g * n, n), n)

        def copy(kind, br, i, half=0, src=None):
            x, k, v, wq, wo = srcs[br if src is None else src]
            if kind == "x":
                return pltpu.make_async_copy(x.at[pl.ds(i * R, R)], xb.at[br, pl.ds(i * R, R)], xsem.at[br, i])
            if kind in "kv":
                hbm, dst = (k, kb) if kind == "k" else (v, vb)
                rows = pl.ds(half * (B // 2), B // 2)
                return pltpu.make_async_copy(hbm.at[rows, heads(i, 2 * NB)], dst.at[br * NSTEP + i, rows],
                                             kvsem.at[br * NSTEP + i, 2 * "kv".index(kind) + half])
            if kind == "q":
                return pltpu.make_async_copy(wq.at[:, heads(i, D)], wqb.at[br * NQUAD + i], wsem.at[br, i])
            return pltpu.make_async_copy(wo.at[heads(i, 2 * D)], wob.at[br * NSTEP + i], wsem.at[br, NQUAD + i])

        def step_copies(br, t, src=None):
            return ([copy("q", br, 2 * t + 1, src=src)] + [copy(kind, br, t, 0, src) for kind in "kv"]
                    + [copy("o", br, t, src=src)] + [copy(kind, br, t, 1, src) for kind in "kv"])

        def out_copy(br, c):
            return pltpu.make_async_copy(ob.at[br, pl.ds(c * R, R)], out.at[pl.ds(c * R, R), heads(br, D)], osem.at[br, c])

        def rows16(ref, idx):
            return pltpu.bitcast(ref.bitcast(u32)[idx], bf16)

        def put(ref, idx, v, as_words):
            ref[idx] = pltpu.bitcast(v.astype(bf16), u32) if as_words else v.astype(bf16)

        def get(ref, idx, as_words):
            return pltpu.bitcast(ref[idx], bf16) if as_words else rows16(ref, idx)

        def weight_operand(ref, slot, row0, p):
            def block(ij):
                return ref[slot, row0 + ij[0] * T:row0 + (ij[0] + 1) * T, ij[1] * T:(ij[1] + 1) * T]

            def signed_sum(terms):
                if len(terms) == 1:
                    return block(terms[0][0]).astype(f32), terms[0][1]
                (u, su), (v, sv) = signed_sum(terms[:len(terms) // 2]), signed_sum(terms[len(terms) // 2:])
                return (u + v, su) if su == sv else ((u - v, 1) if su > 0 else (v - u, 1))

            if len(W_TERMS[p]) == 1:
                return block(W_TERMS[p][0][0])
            total, sign = signed_sum(W_TERMS[p])
            assert sign > 0
            return total

        def x_operands(br, c):
            x = [[xb[br, c * R + i * S:c * R + (i + 1) * S, j * T:(j + 1) * T].astype(f32) for j in range(NB)] for i in range(NB)]
            for p, v in enumerate(left_operands(x)):
                put(xc, (br, c, p), v, True)

        def run(tasks, s, now, then, first=False, last=False, new_x=False, hooks=(), group=None):
            br, t = now
            q_of = {1: (br, 2 * t + 1), 2: (then[0], 2 * then[1]) if group is None else (0, group)}
            hooks, x_done = dict(hooks), set()
            wq_ops, wo_ops, q_prod, q_val, probs, heads_out, o_ops, o_prod = {}, {}, {}, {}, {}, {}, {}, {}
            for task in tasks:
                if task in hooks:
                    hooks[task]()
                kind, c = task[:2]
                if kind == "Q":
                    u, p = task[2:]
                    xbr, g = q_of[u]
                    if new_x and u == 2 and c not in x_done:
                        x_done.add(c)
                        x_operands(xbr, c)
                    if (u, p) not in wq_ops:
                        wq_ops[u, p] = weight_operand(wqb, xbr * NQUAD + g, 0, p).astype(bf16)
                    q_prod[c, u, p] = jnp.dot(get(xc, (xbr, c, p), True), wq_ops[u, p], preferred_element_type=f32)
                elif kind == "q":
                    u = task[2]
                    q = combine([q_prod[c, u, p] for p in range(NP)])
                    for i in range(NB):
                        for h in range(NB):
                            if u == 1:
                                q_val[c, i, h] = q[i][h].astype(bf16)
                            else:
                                put(qb, ((s + 1) % 2 if group is None else 2 * group, c * NB + i, h), q[i][h], False)
                elif kind == "K":
                    for j in range(task[2], task[2] + NB):
                        u, i, h = j // (NB * NB), j // NB % NB, j % NB
                        q = q_val[c, i, h] if u and q_val else get(qb, (2 if u else s % 2, c * NB + i, h), False)
                        k = rows16(kb, (br * NSTEP + t, c * NB + i, u * NB + h))
                        sim = jax.lax.dot_general(q, k, (((1,), (1,)), ((), ())), preferred_element_type=f32)
                        e = jnp.exp2((sim - jnp.max(sim, axis=-1, keepdims=True)) * (DH ** -0.5 * LOG2E))
                        probs[c, j] = (e * pl.reciprocal(jnp.sum(e, axis=-1, keepdims=True), approx=True)).astype(bf16)
                elif kind == "P":
                    for j in range(task[2], task[2] + NB):
                        u, i, h = j // (NB * NB), j // NB % NB, j % NB
                        v = rows16(vb, (br * NSTEP + t, c * NB + i, u * NB + h))
                        heads_out[c, u, i, h] = jnp.dot(probs[c, j], v, preferred_element_type=f32)
                elif kind == "o":
                    ops = [left_operands([[heads_out[c, u, i, h] for h in range(NB)] for i in range(NB)]) for u in range(2)]
                    o_ops[c] = [jnp.concatenate(pair, axis=1).astype(bf16) for pair in zip(*ops)]
                elif kind == "O":
                    p = task[2]
                    if p not in wo_ops:
                        wo_ops[p] = jnp.concatenate([weight_operand(wob, br * NSTEP + t, u * D, p) for u in range(2)], axis=0).astype(bf16)
                    r = jnp.dot(o_ops[c][p], wo_ops[p], preferred_element_type=f32)
                    if not first:
                        r = r + acc[br, c, p]
                    if last:
                        o_prod[c, p] = r
                    else:
                        acc[br, c, p] = r
                elif last:
                    res = combine([o_prod[c, p] for p in range(NP)])
                    for i in range(NB):
                        for j in range(NB):
                            ob[br, c * R + i * S:c * R + (i + 1) * S, j * T:(j + 1) * T] = res[i][j].astype(bf16)
                    out_copy(br, c).start()

        def wait(cps, then=()):
            def hook():
                for cp in cps:
                    cp.wait()
                for cp in then:
                    cp.start()
            return hook

        x = [[copy("x", br, c) for c in range(NC)] for br in range(2)]
        seq = [(0, 0), (0, 1), (1, 0), (0, 2), (1, 1), (1, 2), (0, 3), (1, 3)]
        steps = [step_copies(br, t) for br, t in seq]
        lead = [copy("q", br, 2 * t) for br, t in seq]

        for cp in x[0] + [lead[0]]:
            cp.start()
        for c, then in enumerate(([], [], steps[0][:1], steps[0][1:3] + [lead[1], steps[0][3]])):
            wait([x[0][c]], then)()
            x_operands(0, c)

        def project(g, carry):
            wait([copy("q", 0, g)])()
            run(order((2,), False), 0, seq[0], seq[1], group=g)
            return carry
        jax.lax.fori_loop(0, 2, project, 0)
        wait(steps[0][1:3] + [lead[1]], steps[0][4:] + steps[1][:2])()
        run(order((2,), True, **F), 0, seq[0], seq[1], first=True, hooks={
            ("o", 0): wait(steps[0][3:4], steps[1][2:4]),
            ("K", NC // 2, 0): wait(steps[0][4:], x[1] + [lead[2]])})
        wait(steps[1][:4], steps[1][4:] + steps[2][:2])()
        tasks = order((1, 2), True, **M1)
        needs_late_data = [task for task in tasks if task[0] == "Q" and task[2] == 2 or task[:2] == ("K", NC // 2)]
        run(tasks, 1, seq[1], seq[2], new_x=True,
            hooks={needs_late_data[0]: wait(x[1] + [lead[2]] + steps[1][4:], steps[2][2:] + [lead[3]])})
        wait(steps[2] + [lead[3]], steps[3] + [lead[4]])()
        run(order((1, 2), True, **FB), 2, seq[2], seq[3], first=True)

        def middle(s, carry):
            now = jnp.int32(s >= 4), 2 - jnp.int32(s == 4)
            then = jnp.int32(s < 5), s - 2
            wait(step_copies(*now, src=0) + [copy("q", then[0], 2 * then[1], src=0)])()
            for at, cps in ((3, steps[4] + [lead[5]] + steps[5][:2]), (4, steps[5][2:] + [lead[6]] + steps[6][:4]),
                            (5, steps[6][4:] + [lead[7]] + steps[7])):
                @pl.when(s == at)
                def _():
                    for cp in cps:
                        cp.start()
            run(order((1, 2), True), s, now, then)
            return carry
        jax.lax.fori_loop(3, 6, middle, 0)
        wait(steps[6] + [lead[7]])()
        run(order((1, 2), True, **LA), 6, seq[6], seq[7], last=True)
        wait(steps[7])()
        run(order((1,), True, **L), 7, seq[7], seq[7], last=True)
        for br in range(2):
            for c in range(NC):
                out_copy(br, c).wait()

    def fn(ax, ak, av, awq, awo, bx, bk, bv, bwq, bwo):
        words = lambda shape, w: pltpu.VMEM(shape[:-2] + (shape[-2] // 2, shape[-1]), u32) if w else pltpu.VMEM(shape, bf16)
        out = pl.pallas_call(
            kernel,
            out_shape=jax.ShapeDtypeStruct((M, 2 * D), bf16),
            in_specs=[pl.BlockSpec(memory_space=pl.ANY)] * 10,
            out_specs=pl.BlockSpec(memory_space=pl.ANY),
            scratch_shapes=[
                pltpu.VMEM((2, M, D), bf16),
                pltpu.VMEM((2 * NSTEP, B, 2 * NB, SK, DH), bf16), pltpu.VMEM((2 * NSTEP, B, 2 * NB, SK, DH), bf16),
                pltpu.VMEM((2 * NQUAD, D, NB * DH), bf16), pltpu.VMEM((2 * NSTEP, 2 * NB * DH, D), bf16),
                words((2, NC, NP, S, T), True), words((3, B, NB, S, DH), False),
                pltpu.VMEM((2, NC, NP, S, T), f32),
                pltpu.VMEM((2, M, D), bf16),
                pltpu.SemaphoreType.DMA((2, NC)), pltpu.SemaphoreType.DMA((2 * NSTEP, 4)),
                pltpu.SemaphoreType.DMA((2, NQUAD + NSTEP)), pltpu.SemaphoreType.DMA((2, NC)),
            ],
            compiler_params=pltpu.CompilerParams(
                vmem_limit_bytes=116 * 1024 * 1024, disable_bounds_checks=True),
        )(ax.reshape(M, D), ak, av, awq, awo, bx.reshape(M, D), bk, bv, bwq, bwo)
        return out.reshape(B, S, 2 * D)
    return fn


@jax.jit
def pallas_concat_heads__mha_block_cached__mha_block_cached__near_ridge_kernel(
    A_x, A_k_cache, A_v_cache, A_wq, A_wo, B_x, B_k_cache, B_v_cache, B_wq, B_wo,
):
    return build()(A_x, A_k_cache, A_v_cache, A_wq, A_wo, B_x, B_k_cache, B_v_cache, B_wq, B_wo)
```

```python
import jax
import jax.numpy as jnp
import jax.experimental.pallas as pl
import jax.experimental.pallas.tpu as pltpu

B, S, D, H, SK, DH = 16, 80, 512, 32, 80, 128
M = B * S
T = 128
NB = 4
NC = B // NB
R = NB * S
NQUAD = H // NB
NSTEP = NQUAD // 2
NP = 49
LOG2E = 1.4426950408889634
f32, bf16, u32 = jnp.float32, jnp.bfloat16, jnp.uint32


def _quad(m):
    n = len(m) // 2
    return ([r[:n] for r in m[:n]], [r[n:] for r in m[:n]], [r[:n] for r in m[n:]], [r[n:] for r in m[n:]])


def _add(a, b):
    return [[x + y for x, y in zip(r, s)] for r, s in zip(a, b)]


def _sub(a, b):
    return [[x - y for x, y in zip(r, s)] for r, s in zip(a, b)]


def left_operands(m):
    if len(m) == 1:
        return [m[0][0]]
    a11, a12, a21, a22 = _quad(m)
    parts = (_add(a11, a22), _add(a21, a22), a11, a22, _add(a11, a12), _sub(a21, a11), _sub(a12, a22))
    return [x for t in parts for x in left_operands(t)]


def right_operands(m):
    if len(m) == 1:
        return [m[0][0]]
    b11, b12, b21, b22 = _quad(m)
    parts = (_add(b11, b22), b11, _sub(b12, b22), _sub(b21, b11), b22, _add(b11, b12), _add(b21, b22))
    return [x for t in parts for x in right_operands(t)]


def combine(ps):
    if len(ps) == 1:
        return [[ps[0]]]
    n = len(ps) // 7
    m1, m2, m3, m4, m5, m6, m7 = [combine(ps[i * n:(i + 1) * n]) for i in range(7)]
    c11 = _add(_sub(_add(m1, m4), m5), m7)
    c12 = _add(m3, m5)
    c21 = _add(m2, m4)
    c22 = _add(_add(_sub(m1, m2), m3), m6)
    return [r + s for r, s in zip(c11, c12)] + [r + s for r, s in zip(c21, c22)]


class _Terms:
    def __init__(self, t):
        self.t = t

    def __add__(self, o):
        return _Terms({**self.t, **o.t})

    def __sub__(self, o):
        return _Terms({**self.t, **{k: -v for k, v in o.t.items()}})


W_TERMS = [sorted(x.t.items()) for x in right_operands([[_Terms({(i, j): 1}) for j in range(NB)] for i in range(NB)])]


def product_order(spec):
    d = [int(ch) - 1 for ch in str(spec)]
    return [7 * a + b for a in d for b in d]


def issue_order(q_groups, attend, lagp, lago, tail, gq, go, pq, po, skew, spanf):
    qs = [("Q", c, u, p) for u in q_groups for c in range(NC) for p in product_order(pq)]
    ev = []
    if attend:
        total = 20 * (len(qs) + 2 * NC * NP + 4 * B * NB)
        t0 = skew
        period = (total - t0 - 40 * NP - tail) / NC
        n = 2 * NB * NB // NB
        for c in range(NC):
            for j in range(n):
                at = t0 + (c + j / n) * period
                ev.append((at, 20 * NB, ("K", c, j * NB)))
                ev.append((at + lagp, 20 * NB, ("P", c, j * NB)))
            done = t0 + (c + 1 - 1 / n) * period + lagp
            ev.append((done + 1, 0, ("o", c)))
            span = spanf * period if c < NC - 1 else 40 * NP
            for rank, p in enumerate(product_order(po)):
                ev.append((done + lago + (rank + 0.5) / NP * span, 40, ("O", c, p)))
            ev.append((done + lago + span, 0, ("F", c)))
    ev.sort(key=lambda e: e[0])
    out, held, cum = [], [], 0

    def emit_q():
        t = qs.pop(0)
        out.append(t)
        if not qs or qs[0][1:3] != t[1:3]:
            out.append(("q",) + t[1:3])

    for at, cost, t in ev:
        while len(qs) >= gq and cum + 10 * gq <= at:
            for _ in range(gq):
                emit_q()
            cum += 20 * gq
        if t[0] == "K" and t[2] >= NB * NB:
            while 1 in q_groups and ("q", t[1], 1) not in out:
                emit_q()
                cum += 20
        if t[0] == "O" or (held and t[0] == "F"):
            held.append(t)
            if sum(h[0] == "O" for h in held) == go:
                out += held
                held = []
                cum += 40 * go
        else:
            out.append(t)
            cum += cost
    while qs:
        emit_q()
    return out + held


PLAIN = dict(lagp=600, lago=650, tail=3300, gq=1, go=1, pq=3524167, po=3425671, skew=0, spanf=1.1)
F = dict(lagp=600, lago=200, tail=1200, spanf=1.2)
M1 = dict(lagp=600, lago=500, tail=3800, go=2, spanf=1.0)
FB = dict(lagp=600, lago=500, tail=3800, go=2, pq=2413567, spanf=1.2)
LA = dict(lagp=600, lago=300, tail=2200, gq=2, go=2, pq=2413567, spanf=1.0, skew=200)
L = dict(lagp=550, lago=300, tail=-600, gq=2, go=2, pq=2413567, spanf=1.0)


def order(q_groups, attend, **kw):
    return issue_order(q_groups, attend, **{**PLAIN, **kw})


def build():
    def kernel(ax, ak, av, awq, awo, bx, bk, bv, bwq, bwo, out,
               xb, kb, vb, wqb, wob, xc, qb, acc, ob, xsem, kvsem, wsem, osem):
        srcs = ((ax, ak, av, awq, awo), (bx, bk, bv, bwq, bwo))

        def heads(g, n):
            return pl.ds(g * n if isinstance(g, int) else pl.multiple_of(g * n, n), n)

        def copy(kind, br, i, half=0, src=None):
            x, k, v, wq, wo = srcs[br if src is None else src]
            if kind == "x":
                return pltpu.make_async_copy(x.at[pl.ds(i * R, R)], xb.at[br, pl.ds(i * R, R)], xsem.at[br, i])
            if kind in "kv":
                hbm, dst = (k, kb) if kind == "k" else (v, vb)
                rows = pl.ds(half * (B // 2), B // 2)
                return pltpu.make_async_copy(hbm.at[rows, heads(i, 2 * NB)], dst.at[br * NSTEP + i, rows],
                                             kvsem.at[br * NSTEP + i, 2 * "kv".index(kind) + half])
            if kind == "q":
                return pltpu.make_async_copy(wq.at[:, heads(i, D)], wqb.at[br * NQUAD + i], wsem.at[br, i])
            return pltpu.make_async_copy(wo.at[heads(i, 2 * D)], wob.at[br * NSTEP + i], wsem.at[br, NQUAD + i])

        def step_copies(br, t, src=None):
            return ([copy("q", br, 2 * t + 1, src=src)] + [copy(kind, br, t, 0, src) for kind in "kv"]
                    + [copy("o", br, t, src=src)] + [copy(kind, br, t, 1, src) for kind in "kv"])

        def out_copy(br, c):
            return pltpu.make_async_copy(ob.at[br, pl.ds(c * R, R)], out.at[pl.ds(c * R, R), heads(br, D)], osem.at[br, c])

        def rows16(ref, idx):
            return pltpu.bitcast(ref.bitcast(u32)[idx], bf16)

        def put(ref, idx, v, as_words):
            ref[idx] = pltpu.bitcast(v.astype(bf16), u32) if as_words else v.astype(bf16)

        def get(ref, idx, as_words):
            return pltpu.bitcast(ref[idx], bf16) if as_words else rows16(ref, idx)

        def weight_operand(ref, slot, row0, p):
            def block(ij):
                return ref[slot, row0 + ij[0] * T:row0 + (ij[0] + 1) * T, ij[1] * T:(ij[1] + 1) * T]

            def signed_sum(terms):
                if len(terms) == 1:
                    return block(terms[0][0]).astype(f32), terms[0][1]
                (u, su), (v, sv) = signed_sum(terms[:len(terms) // 2]), signed_sum(terms[len(terms) // 2:])
                return (u + v, su) if su == sv else ((u - v, 1) if su > 0 else (v - u, 1))

            if len(W_TERMS[p]) == 1:
                return block(W_TERMS[p][0][0])
            total, sign = signed_sum(W_TERMS[p])
            assert sign > 0
            return total

        def x_operands(br, c):
            x = [[xb[br, c * R + i * S:c * R + (i + 1) * S, j * T:(j + 1) * T].astype(f32) for j in range(NB)] for i in range(NB)]
            for p, v in enumerate(left_operands(x)):
                put(xc, (br, c, p), v, as_words=True)

        def run(tasks, s, now, then, first=False, last=False, new_x=False, hooks=(), group=None):
            br, t = now
            q_of = {1: (br, 2 * t + 1), 2: (then[0], 2 * then[1]) if group is None else (0, group)}
            hooks, x_done = dict(hooks), set()
            wq_ops, wo_ops, q_prod, q_val, probs, heads_out, o_ops, o_prod = {}, {}, {}, {}, {}, {}, {}, {}
            for task in tasks:
                if task in hooks:
                    hooks[task]()
                kind, c = task[:2]
                if kind == "Q":
                    u, p = task[2:]
                    xbr, g = q_of[u]
                    if new_x and u == 2 and c not in x_done:
                        x_done.add(c)
                        x_operands(xbr, c)
                    if (u, p) not in wq_ops:
                        wq_ops[u, p] = weight_operand(wqb, xbr * NQUAD + g, 0, p).astype(bf16)
                    q_prod[c, u, p] = jnp.dot(get(xc, (xbr, c, p), as_words=True), wq_ops[u, p], preferred_element_type=f32)
                elif kind == "q":
                    u = task[2]
                    q = combine([q_prod[c, u, p] for p in range(NP)])
                    for i in range(NB):
                        for h in range(NB):
                            if u == 1:
                                q_val[c, i, h] = q[i][h].astype(bf16)
                            else:
                                put(qb, ((s + 1) % 2 if group is None else 2 * group, c * NB + i, h), q[i][h], as_words=False)
                elif kind == "K":
                    for j in range(task[2], task[2] + NB):
                        u, i, h = j // (NB * NB), j // NB % NB, j % NB
                        q = q_val[c, i, h] if u and q_val else get(qb, (2 if u else s % 2, c * NB + i, h), as_words=False)
                        k = rows16(kb, (br * NSTEP + t, c * NB + i, u * NB + h))
                        sim = jax.lax.dot_general(q, k, (((1,), (1,)), ((), ())), preferred_element_type=f32)
                        e = jnp.exp2((sim - jnp.max(sim, axis=-1, keepdims=True)) * (DH ** -0.5 * LOG2E))
                        probs[c, j] = (e * pl.reciprocal(jnp.sum(e, axis=-1, keepdims=True), approx=True)).astype(bf16)
                elif kind == "P":
                    for j in range(task[2], task[2] + NB):
                        u, i, h = j // (NB * NB), j // NB % NB, j % NB
                        v = rows16(vb, (br * NSTEP + t, c * NB + i, u * NB + h))
                        heads_out[c, u, i, h] = jnp.dot(probs[c, j], v, preferred_element_type=f32)
                elif kind == "o":
                    ops = [left_operands([[heads_out[c, u, i, h] for h in range(NB)] for i in range(NB)]) for u in range(2)]
                    o_ops[c] = [jnp.concatenate(pair, axis=1).astype(bf16) for pair in zip(*ops)]
                elif kind == "O":
                    p = task[2]
                    if p not in wo_ops:
                        wo_ops[p] = jnp.concatenate([weight_operand(wob, br * NSTEP + t, u * D, p) for u in range(2)], axis=0).astype(bf16)
                    r = jnp.dot(o_ops[c][p], wo_ops[p], preferred_element_type=f32)
                    if not first:
                        r = r + acc[br, c, p]
                    if last:
                        o_prod[c, p] = r
                    else:
                        acc[br, c, p] = r
                elif last:
                    res = combine([o_prod[c, p] for p in range(NP)])
                    for i in range(NB):
                        for j in range(NB):
                            ob[br, c * R + i * S:c * R + (i + 1) * S, j * T:(j + 1) * T] = res[i][j].astype(bf16)
                    out_copy(br, c).start()

        def wait(cps, then=()):
            def hook():
                for cp in cps:
                    cp.wait()
                for cp in then:
                    cp.start()
            return hook

        x = [[copy("x", br, c) for c in range(NC)] for br in range(2)]
        seq = [(0, 0), (0, 1), (1, 0), (0, 2), (1, 1), (1, 2), (0, 3), (1, 3)]
        steps = [step_copies(br, t) for br, t in seq]
        lead = [copy("q", br, 2 * t) for br, t in seq]

        for cp in x[0] + [lead[0]]:
            cp.start()
        for c, then in enumerate(([], [], steps[0][:1], steps[0][1:3] + [lead[1], steps[0][3]])):
            wait([x[0][c]], then)()
            x_operands(0, c)

        def project(g, carry):
            wait([copy("q", 0, g)])()
            run(order((2,), False), 0, seq[0], seq[1], group=g)
            return carry
        jax.lax.fori_loop(0, 2, project, 0)
        wait(steps[0][1:3] + [lead[1]], steps[0][4:] + steps[1][:2])()
        run(order((2,), True, **F), 0, seq[0], seq[1], first=True, hooks={
            ("o", 0): wait(steps[0][3:4], steps[1][2:4]),
            ("K", NC // 2, 0): wait(steps[0][4:], x[1] + [lead[2]])})
        wait(steps[1][:4], steps[1][4:] + steps[2][:2])()
        tasks = order((1, 2), True, **M1)
        needs_late_data = [task for task in tasks if task[0] == "Q" and task[2] == 2 or task[:2] == ("K", NC // 2)]
        run(tasks, 1, seq[1], seq[2], new_x=True,
            hooks={needs_late_data[0]: wait(x[1] + [lead[2]] + steps[1][4:], steps[2][2:] + [lead[3]])})
        wait(steps[2] + [lead[3]], steps[3] + [lead[4]])()
        run(order((1, 2), True, **FB), 2, seq[2], seq[3], first=True)

        def middle(s, carry):
            now = jnp.int32(s >= 4), 2 - jnp.int32(s == 4)
            then = jnp.int32(s < 5), s - 2
            wait(step_copies(*now, src=0) + [copy("q", then[0], 2 * then[1], src=0)])()
            for at, cps in ((3, steps[4] + [lead[5]] + steps[5][:2]), (4, steps[5][2:] + [lead[6]] + steps[6][:4]),
                            (5, steps[6][4:] + [lead[7]] + steps[7])):
                @pl.when(s == at)
                def _():
                    for cp in cps:
                        cp.start()
            run(order((1, 2), True), s, now, then)
            return carry
        jax.lax.fori_loop(3, 6, middle, 0)
        wait(steps[6] + [lead[7]])()
        run(order((1, 2), True, **LA), 6, seq[6], seq[7], last=True)
        wait(steps[7])()
        run(order((1,), True, **L), 7, seq[7], seq[7], last=True)
        for br in range(2):
            for c in range(NC):
                out_copy(br, c).wait()

    def fn(ax, ak, av, awq, awo, bx, bk, bv, bwq, bwo):
        words = lambda shape, w: pltpu.VMEM(shape[:-2] + (shape[-2] // 2, shape[-1]), u32) if w else pltpu.VMEM(shape, bf16)
        out = pl.pallas_call(
            kernel,
            out_shape=jax.ShapeDtypeStruct((M, 2 * D), bf16),
            in_specs=[pl.BlockSpec(memory_space=pl.ANY)] * 10,
            out_specs=pl.BlockSpec(memory_space=pl.ANY),
            scratch_shapes=[
                pltpu.VMEM((2, M, D), bf16),
                pltpu.VMEM((2 * NSTEP, B, 2 * NB, SK, DH), bf16), pltpu.VMEM((2 * NSTEP, B, 2 * NB, SK, DH), bf16),
                pltpu.VMEM((2 * NQUAD, D, NB * DH), bf16), pltpu.VMEM((2 * NSTEP, 2 * NB * DH, D), bf16),
                words((2, NC, NP, S, T), True), words((3, B, NB, S, DH), False),
                pltpu.VMEM((2, NC, NP, S, T), f32),
                pltpu.VMEM((2, M, D), bf16),
                pltpu.SemaphoreType.DMA((2, NC)), pltpu.SemaphoreType.DMA((2 * NSTEP, 4)),
                pltpu.SemaphoreType.DMA((2, NQUAD + NSTEP)), pltpu.SemaphoreType.DMA((2, NC)),
            ],
            compiler_params=pltpu.CompilerParams(
                vmem_limit_bytes=116 * 1024 * 1024, disable_bounds_checks=True),
        )(ax.reshape(M, D), ak, av, awq, awo, bx.reshape(M, D), bk, bv, bwq, bwo)
        return out.reshape(B, S, 2 * D)
    return fn


@jax.jit
def pallas_concat_heads__mha_block_cached__mha_block_cached__near_ridge_kernel(
    A_x, A_k_cache, A_v_cache, A_wq, A_wo, B_x, B_k_cache, B_v_cache, B_wq, B_wo,
):
    return build()(A_x, A_k_cache, A_v_cache, A_wq, A_wo, B_x, B_k_cache, B_v_cache, B_wq, B_wo)
```
